```python
import os as _os
_os.environ.setdefault("JAX_PLATFORMS", "cpu")
import jax
import jax.numpy as jnp

def _softmax(x, axis=-1):
    return jax.nn.softmax(x, axis=axis)
def _gelu(x):
    return jax.nn.gelu(x, approximate=True)
def _silu(x):
    return jax.nn.silu(x)
def _sigmoid(x):
    return jax.nn.sigmoid(x)
def _layernorm(x, axis=-1, eps=1e-5):
    m = jnp.mean(x, axis=axis, keepdims=True)
    v = jnp.var(x, axis=axis, keepdims=True)
    return (x - m) / jnp.sqrt(v + eps)
def _scatter_add(tgt, idx, src, axis=0):
    return tgt.at[idx].add(src)
def _segment_sum(src, seg, n):
    return jax.ops.segment_sum(src, seg, n)
class _Rng:
    def __init__(self, key):
        self._k = key
    def _next(self):
        self._k, sub = jax.random.split(self._k)
        return sub
    def normal(self, shape):
        return jax.random.normal(self._next(), shape, dtype=jnp.bfloat16)
    def randint(self, lo, hi, shape):
        return jax.random.randint(self._next(), shape, lo, hi, dtype=jnp.int32)
    def uniform(self, shape, lo=0.0, hi=1.0):
        return jax.random.uniform(self._next(), shape, jnp.bfloat16, lo, hi)
    def permutation(self, n):
        return jax.random.permutation(self._next(), n)


kernel_name = 'standalone__gqa_block_cached__near_ridge'

def setup_inputs():
    _rng = _Rng(jax.random.key(int.from_bytes(__import__("os").urandom(4), "little")))
    _w = (lambda a: (lambda t: t.astype(jnp.bfloat16) if jnp.issubdtype(t.dtype, jnp.floating) else t)(jnp.asarray(a)))
    B, Sq, D = 8, 80, 512
    Hq, Hkv, Sk, Dh = 32, 8, 2048, 128
    assert Hq % Hkv == 0, (Hq, Hkv)
    return {
        "x": _w((lambda *s: _rng.normal(s) * 0.8)(B, Sq, D)),
        "k_cache": _w((lambda *s: _rng.normal(s) * 0.8)(B, Hkv, Sk, Dh)),
        "v_cache": _w((lambda *s: _rng.normal(s) * 0.05)(B, Hkv, Sk, Dh)),
        "wq": _w((lambda *s: _rng.normal(s) * 0.8)(D, Hq * Dh) * (D ** -0.5)),
        "wo": _w((lambda *s: _rng.normal(s) * 0.05)(Hq * Dh, D) * ((Hq * Dh) ** -0.5)),
    }

def reference(x, k_cache, v_cache, wq, wo):
    B, Sq, D = x.shape
    Hq, Dh = 32, 128
    Hkv = k_cache.shape[1]
    rep = Hq // Hkv
    q = (lambda x, *d: x.transpose(*d))((x @ wq).reshape(B, Sq, Hq, Dh), 0, 2, 1, 3)
    k = jnp.repeat(k_cache, rep, axis=1)
    v = jnp.repeat(v_cache, rep, axis=1)
    scores = jnp.einsum("bhqd,bhkd->bhqk", q, k) * (Dh ** -0.5)
    p = _softmax(scores, axis=-1)
    o = jnp.einsum("bhqk,bhkd->bhqd", p, v)
    return (lambda x, *d: x.transpose(*d))(o, 0, 2, 1, 3).reshape(B, Sq, Hq * Dh) @ wo
```

```python
import functools
import jax
import jax.numpy as jnp
from jax import lax
import jax.experimental.pallas as pl
import jax.experimental.pallas.tpu as pltpu

LOG2E = 1.4426950408889634
NT = (((1,), (1,)), ((), ()))


def build(N=2, RG=3, TK=512, DPOS=1, DSPLIT=True):
    def fn(x, k_cache, v_cache, wq, wo):
        B, Sq, D = x.shape
        _, Hkv, Sk, Dh = k_cache.shape
        Hq = wq.shape[1] // Dh
        rep = Hq // Hkv
        G = rep * Dh
        M = rep * Sq
        U = B * Hkv
        NC = Sk // TK
        LT = TK // 128
        scale = (Dh ** -0.5) * LOG2E
        assert Hkv % N == 0
        NB = U // N
        assert NB % 2 == 0
        x2 = x.reshape(B * Sq, D)
        k4 = k_cache.reshape(NB, N, Sk, Dh)
        v4 = v_cache.reshape(NB, N, Sk, Dh)

        def kernel(x_hbm, k_hbm, v_hbm, wq_hbm, wo_hbm, out_ref,
                   x_v, wq_v, wo_v, k_buf, v_buf, q_scr, s0, s1, m0, m1, oa0, oa1, la0, la1, acc_scr,
                   sem_x, sem_wq, sem_wo, sem_k, sem_v):
            s_bufs = (s0, s1)
            m_bufs = (m0, m1)
            o_bufs = (oa0, oa1)
            l_bufs = (la0, la1)

            def x_copy():
                return pltpu.make_async_copy(x_hbm, x_v, sem_x.at[0])

            def wq_copy(h):
                return pltpu.make_async_copy(wq_hbm.at[:, pl.ds(h * G, G)], wq_v.at[h], sem_wq.at[h])

            def wo_copy(h):
                return pltpu.make_async_copy(wo_hbm.at[pl.ds(h * G, G), :], wo_v.at[pl.ds(h * G, G), :], sem_wo.at[h])

            def k_copy(j):
                return pltpu.make_async_copy(k_hbm.at[j], k_buf.at[j % RG], sem_k.at[j % RG])

            def v_copy(j):
                return pltpu.make_async_copy(v_hbm.at[j], v_buf.at[j % RG], sem_v.at[j % RG])

            x_copy().start()
            wq_copy(0).start()
            wq_copy(1).start()
            acc_scr[...] = jnp.zeros(acc_scr.shape, jnp.float32)
            x_copy().wait()

            def qproj(h):
                q = jnp.dot(x_v[...], wq_v[h], preferred_element_type=jnp.float32)
                q = (q * scale).astype(jnp.bfloat16)
                for bb in range(B):
                    for r in range(rep):
                        q_scr[bb * Hkv + h, r * Sq:(r + 1) * Sq, :] = q[bb * Sq:(bb + 1) * Sq, r * Dh:(r + 1) * Dh]

            def p1_body(h, c):
                wq_copy(h).wait()

                @pl.when(h + 2 < Hkv)
                def _():
                    wq_copy(h + 2).start()

                @pl.when(h == 2)
                def _():
                    k_copy(0).start()

                @pl.when(h == 4)
                def _():
                    k_copy(1).start()

                @pl.when(h == 6)
                def _():
                    v_copy(0).start()

                wo_copy(h).start()
                qproj(h)
                return c

            lax.fori_loop(0, Hkv, p1_body, 0)
            for j in range(2, RG):
                k_copy(j).start()
            for j in range(1, RG):
                v_copy(j).start()

            def b_chunk(j, i, par, c, mrun):
                q = q_scr[j * N + i]
                s = lax.dot_general(q, k_buf[j % RG, i, c * TK:(c + 1) * TK, :], NT, preferred_element_type=jnp.float32)
                s_bufs[par][i, :, c * TK:(c + 1) * TK] = s
                t = s[:, 0:128]
                for ii in range(1, LT):
                    t = jnp.maximum(t, s[:, ii * 128:(ii + 1) * 128])
                mrun = t if mrun is None else jnp.maximum(mrun, t)
                if c == NC - 1:
                    m = jnp.max(mrun, axis=1, keepdims=True)
                    m_bufs[par][i] = jnp.broadcast_to(m, (M, 128))
                return mrun

            def c_chunk(j, i, par, c, carry):
                lrun, acc = carry
                m = m_bufs[par][i]
                mt = jnp.concatenate([m] * LT, axis=1)
                p = jnp.exp2(s_bufs[par][i, :, c * TK:(c + 1) * TK] - mt)
                t = p[:, 0:128]
                for ii in range(1, LT):
                    t = t + p[:, ii * 128:(ii + 1) * 128]
                lrun = t if lrun is None else lrun + t
                pv = jnp.dot(p.astype(jnp.bfloat16), v_buf[j % RG, i, c * TK:(c + 1) * TK, :], preferred_element_type=jnp.float32)
                acc = pv if acc is None else pv + acc
                if c == NC - 1:
                    o_bufs[par][i] = acc
                    l_bufs[par][i] = lrun
                return lrun, acc

            def stage_d(j, par, units):
                u0 = j * N
                b = u0 // Hkv
                h0 = u0 % Hkv + units[0]
                parts = []
                for i in units:
                    l = jnp.sum(l_bufs[par][i], axis=1, keepdims=True)
                    r0 = pl.reciprocal(l, approx=True)
                    r = r0 * (2.0 - l * r0)
                    o = (o_bufs[par][i] * r).astype(jnp.bfloat16)
                    for rr in range(rep):
                        parts.append(o[rr * Sq:(rr + 1) * Sq, :])
                o = jnp.concatenate(parts, axis=1)
                w = wo_v[pl.ds(pl.multiple_of(h0 * G, G), len(units) * G), :]
                y = jnp.dot(o, w, preferred_element_type=jnp.float32)
                rows = pl.ds(pl.multiple_of(b * Sq, 16), Sq)
                acc_scr[rows, :] += y

            def body(j, par, first=False, last=False):
                v_copy(j).wait()
                if not last:
                    k_copy(j + 1).wait()
                if not last:
                    if not first:
                        @pl.when(j - 1 + RG < NB)
                        def _():
                            v_copy(j - 1 + RG).start()

                    @pl.when(j + RG < NB)
                    def _():
                        k_copy(j + RG).start()
                for i in range(N):
                    mrun = None
                    carry = (None, None)
                    for c in range(NC):
                        if not last:
                            mrun = b_chunk(j + 1, i, 1 - par, c, mrun)
                        if not first and c == DPOS:
                            if DSPLIT:
                                stage_d(j - 1, 1 - par, [i])
                            elif i == 0:
                                stage_d(j - 1, 1 - par, list(range(N)))
                        carry = c_chunk(j, i, par, c, carry)

            k_copy(0).wait()
            for i in range(N):
                mrun = None
                for c in range(NC):
                    mrun = b_chunk(0, i, 0, c, mrun)
            for h in range(Hkv):
                wo_copy(h).wait()
            body(0, 0, first=True)

            def loop_body(jj, c):
                body(2 * jj + 1, 1)
                body(2 * jj + 2, 0)
                return c

            lax.fori_loop(0, (NB - 2) // 2, loop_body, 0)
            body(NB - 1, 1, last=True)
            stage_d(NB - 1, 1, list(range(N)))
            out_ref[...] = acc_scr[...].astype(out_ref.dtype)

        out = pl.pallas_call(
            kernel,
            in_specs=[pl.BlockSpec(memory_space=pl.ANY)] * 5,
            out_specs=pl.BlockSpec(memory_space=pltpu.VMEM),
            out_shape=jax.ShapeDtypeStruct((B * Sq, D), x.dtype),
            scratch_shapes=[
                pltpu.VMEM((B * Sq, D), jnp.bfloat16),
                pltpu.VMEM((Hkv, D, G), jnp.bfloat16),
                pltpu.VMEM((Hq * Dh, D), jnp.bfloat16),
                pltpu.VMEM((RG, N, Sk, Dh), jnp.bfloat16),
                pltpu.VMEM((RG, N, Sk, Dh), jnp.bfloat16),
                pltpu.VMEM((U, M, Dh), jnp.bfloat16),
                pltpu.VMEM((N, M, Sk), jnp.float32),
                pltpu.VMEM((N, M, Sk), jnp.float32),
                pltpu.VMEM((N, M, 128), jnp.float32),
                pltpu.VMEM((N, M, 128), jnp.float32),
                pltpu.VMEM((N, M, Dh), jnp.float32),
                pltpu.VMEM((N, M, Dh), jnp.float32),
                pltpu.VMEM((N, M, 128), jnp.float32),
                pltpu.VMEM((N, M, 128), jnp.float32),
                pltpu.VMEM((B * Sq, D), jnp.float32),
                pltpu.SemaphoreType.DMA((1,)),
                pltpu.SemaphoreType.DMA((Hkv,)),
                pltpu.SemaphoreType.DMA((Hkv,)),
                pltpu.SemaphoreType.DMA((RG,)),
                pltpu.SemaphoreType.DMA((RG,)),
            ],
            compiler_params=pltpu.CompilerParams(
                vmem_limit_bytes=100 * 1024 * 1024,
            ),
        )(x2, k4, v4, wq, wo)
        return out.reshape(B, Sq, D)
    return fn


_impl = build(N=2)


@jax.jit
def pallas_standalone__gqa_block_cached__near_ridge_kernel(
    x: jax.Array,
    k_cache: jax.Array,
    v_cache: jax.Array,
    wq: jax.Array,
    wo: jax.Array,
):
    return _impl(x, k_cache, v_cache, wq, wo)
```

```python
import contextlib
import jax
import jax.numpy as jnp
from jax import lax
import jax.experimental.pallas as pl
import jax.experimental.pallas.tpu as pltpu

LOG2E = 1.4426950408889634
NT = (((1,), (1,)), ((), ()))


def build(N=4, TK=512, DPOS=1, QSPLIT=(1, 3, 3), NOBC=True, NOSC=True, SC=False, KPOS=1):
    scope = jax.named_scope if SC else (lambda n: contextlib.nullcontext())

    def fn(x, k_cache, v_cache, wq, wo):
        B, Sq, D = x.shape
        _, Hkv, Sk, Dh = k_cache.shape
        Hq = wq.shape[1] // Dh
        rep = Hq // Hkv
        G = rep * Dh
        M = rep * Sq
        U = B * Hkv
        NC = Sk // TK
        LT = TK // 128
        scale = (Dh ** -0.5) * LOG2E
        assert Hkv % N == 0
        GPB = Hkv // N
        assert GPB in (1, 2)
        NB = U // N
        assert NB % 2 == 0 and sum(QSPLIT) == Hkv - 1
        x2 = x.reshape(B * Sq, D)
        k4 = k_cache.reshape(NB, N, Sk, Dh)
        v4 = v_cache.reshape(NB, N, Sk, Dh)

        def kernel(x_hbm, k_hbm, v_hbm, wq_hbm, wo_hbm, out_hbm,
                   x_v, wq_v, wo_v, kb0, kb1, vb0, vb1, q_scr, s0, s1, m0, m1, oa0, oa1, la0, la1,
                   acc_scr, out_v,
                   sem_x, sem_wq, sem_wo, sem_k, sem_v, sem_o):
            k_bufs = (kb0, kb1)
            v_bufs = (vb0, vb1)
            s_bufs = (s0, s1)
            m_bufs = (m0, m1)
            o_bufs = (oa0, oa1)
            l_bufs = (la0, la1)

            HR = B * Sq // 2
            HG = G // 2

            def x_copy(a):
                return pltpu.make_async_copy(x_hbm.at[pl.ds(a * HR, HR)], x_v.at[pl.ds(a * HR, HR)], sem_x.at[a])

            def wq0_copy(a):
                return pltpu.make_async_copy(wq_hbm.at[:, pl.ds(a * HG, HG)], wq_v.at[0, :, pl.ds(a * HG, HG)], sem_x.at[2 + a])

            def wq_copy(h):
                return pltpu.make_async_copy(wq_hbm.at[:, pl.ds(h * G, G)], wq_v.at[h], sem_wq.at[h])

            HW = Hq * Dh // 2

            def wo_copy(a):
                return pltpu.make_async_copy(wo_hbm.at[pl.ds(a * HW, HW)], wo_v.at[pl.ds(a * HW, HW)], sem_wo.at[a])

            def k_copy(j, par):
                return pltpu.make_async_copy(k_hbm.at[j], k_bufs[par], sem_k.at[par])

            def v_copy(j, par):
                return pltpu.make_async_copy(v_hbm.at[j], v_bufs[par], sem_v.at[par])

            def out_copy(b):
                return pltpu.make_async_copy(out_v.at[b], out_hbm.at[b], sem_o.at[b])

            def qproj(h, b0=0, b1=B, r0=0, r1=rep):
                q = jnp.dot(x_v[b0 * Sq:b1 * Sq, :], wq_v[h, :, r0 * Dh:r1 * Dh], preferred_element_type=jnp.float32)
                q = (q * scale).astype(jnp.bfloat16)
                for bb in range(b0, b1):
                    for r in range(r0, r1):
                        q_scr[bb * Hkv + h, r * Sq:(r + 1) * Sq, :] = q[(bb - b0) * Sq:(bb - b0 + 1) * Sq, (r - r0) * Dh:(r - r0 + 1) * Dh]

            def b_chunk(j, i, par, c, mrun):
                q = q_scr[j * N + i]
                s = lax.dot_general(q, k_bufs[par][i, c * TK:(c + 1) * TK, :], NT, preferred_element_type=jnp.float32)
                s_bufs[par][i, :, c * TK:(c + 1) * TK] = s
                t = s[:, 0:128]
                for ii in range(1, LT):
                    t = jnp.maximum(t, s[:, ii * 128:(ii + 1) * 128])
                mrun = t if mrun is None else jnp.maximum(mrun, t)
                if c == NC - 1:
                    m = jnp.max(mrun, axis=1, keepdims=True)
                    m_bufs[par][i] = jnp.broadcast_to(m, (M, 128))
                return mrun

            def c_chunk(i, par, c, carry):
                lrun, acc = carry
                m = m_bufs[par][i]
                mt = jnp.concatenate([m] * LT, axis=1)
                p = jnp.exp2(s_bufs[par][i, :, c * TK:(c + 1) * TK] - mt)
                t = p[:, 0:128]
                for ii in range(1, LT):
                    t = t + p[:, ii * 128:(ii + 1) * 128]
                lrun = t if lrun is None else lrun + t
                pv = jnp.dot(p.astype(jnp.bfloat16), v_bufs[par][i, c * TK:(c + 1) * TK, :], preferred_element_type=jnp.float32)
                acc = pv if acc is None else pv + acc
                if c == NC - 1:
                    o_bufs[par][i] = acc
                    l_bufs[par][i] = lrun
                return lrun, acc

            def d_unit(par, i, y):
                h = (par % GPB) * N + i
                l = jnp.sum(l_bufs[par][i], axis=1, keepdims=True)
                r0 = pl.reciprocal(l, approx=True)
                r = r0 * (2.0 - l * r0)
                o = (o_bufs[par][i] * r).astype(jnp.bfloat16)
                o = jnp.concatenate([o[rr * Sq:(rr + 1) * Sq, :] for rr in range(rep)], axis=1)
                yi = jnp.dot(o, wo_v[h * G:(h + 1) * G, :], preferred_element_type=jnp.float32)
                return yi if y is None else yi + y

            def d_init(par):
                return acc_scr[...] if (GPB == 2 and par == 1) else None

            def d_finish(j, par, y):
                if GPB == 2 and par == 0:
                    acc_scr[...] = y
                    return False
                out_v[j // GPB] = y.astype(out_v.dtype)
                return True

            def body(j, par, first=False, last=False):
                with scope("bwait"):
                    v_copy(j, par).wait()
                    if not last:
                        k_copy(j + 1, 1 - par).wait()
                y = None if first else d_init(1 - par)
                for i in range(N):
                    mrun = None
                    carry = (None, None)
                    for c in range(NC):
                        if not last:
                            mrun = b_chunk(j + 1, i, 1 - par, c, mrun)
                        if not first and c == DPOS:
                            y = d_unit(1 - par, i, y)
                        carry = c_chunk(i, par, c, carry)
                if not first:
                    if d_finish(j - 1, 1 - par, y):
                        out_copy((j - 1) // GPB).start()
                if not last:
                    @pl.when(j + 2 < NB)
                    def _():
                        v_copy(j + 2, par).start()

                    @pl.when(j + 3 < NB)
                    def _():
                        k_copy(j + 3, 1 - par).start()

            with scope("p0"):
                wq0_copy(0).start()
                x_copy(0).start()
                x_copy(1).start()
                wq0_copy(1).start()
                wq0_copy(0).wait()
                x_copy(0).wait()
            for h in range(1, 3):
                wq_copy(h).start()
            qproj(0, 0, B // 2, 0, rep // 2)
            with scope("qwait"):
                x_copy(1).wait()
            for h in range(3, 5):
                wq_copy(h).start()
            qproj(0, B // 2, B, 0, rep // 2)
            with scope("qwait"):
                wq0_copy(1).wait()
            for h in range(5, Hkv):
                wq_copy(h).start()
            qproj(0, 0, B, rep // 2, rep)
            h0 = 1
            for gi, g in enumerate(QSPLIT):
                lastq = gi == len(QSPLIT) - 1
                with scope("qwait"):
                    for h in range(h0, h0 + g):
                        wq_copy(h).wait()
                    if lastq:
                        k_copy(0, 0).wait()
                if gi == KPOS:
                    k_copy(0, 0).start()
                if gi == 1:
                    k_copy(1, 1).start()
                    v_copy(0, 0).start()
                if lastq:
                    wo_copy(0).start()
                    v_copy(1, 1).start()
                for h in range(h0, h0 + g):
                    qproj(h)
                h0 += g
            for i in range(N):
                mrun = None
                for c in range(NC):
                    mrun = b_chunk(0, i, 0, c, mrun)
            k_copy(2, 0).start()
            wo_copy(1).start()
            body(0, 0, first=True)
            wo_copy(0).wait()
            if GPB == 1:
                wo_copy(1).wait()

            def loop_body(jj, c):
                body(2 * jj + 1, 1)
                if GPB == 2:
                    @pl.when(jj == 0)
                    def _():
                        wo_copy(1).wait()
                body(2 * jj + 2, 0)
                return c

            lax.fori_loop(0, (NB - 2) // 2, loop_body, 0)
            body(NB - 1, 1, last=True)
            y = d_init(1)
            for i in range(N):
                y = d_unit(1, i, y)
            d_finish(NB - 1, 1, y)
            with scope("final"):
                out_copy(B - 1).start()
                for b in range(B):
                    out_copy(b).wait()

        out = pl.pallas_call(
            kernel,
            in_specs=[pl.BlockSpec(memory_space=pl.ANY)] * 5,
            out_specs=pl.BlockSpec(memory_space=pl.ANY),
            out_shape=jax.ShapeDtypeStruct((B, Sq, D), x.dtype),
            scratch_shapes=[
                pltpu.VMEM((B * Sq, D), jnp.bfloat16),
                pltpu.VMEM((Hkv, D, G), jnp.bfloat16),
                pltpu.VMEM((Hq * Dh, D), jnp.bfloat16),
                pltpu.VMEM((N, Sk, Dh), jnp.bfloat16),
                pltpu.VMEM((N, Sk, Dh), jnp.bfloat16),
                pltpu.VMEM((N, Sk, Dh), jnp.bfloat16),
                pltpu.VMEM((N, Sk, Dh), jnp.bfloat16),
                pltpu.VMEM((U, M, Dh), jnp.bfloat16),
                pltpu.VMEM((N, M, Sk), jnp.float32),
                pltpu.VMEM((N, M, Sk), jnp.float32),
                pltpu.VMEM((N, M, 128), jnp.float32),
                pltpu.VMEM((N, M, 128), jnp.float32),
                pltpu.VMEM((N, M, Dh), jnp.float32),
                pltpu.VMEM((N, M, Dh), jnp.float32),
                pltpu.VMEM((N, M, 128), jnp.float32),
                pltpu.VMEM((N, M, 128), jnp.float32),
                pltpu.VMEM((Sq, D), jnp.float32),
                pltpu.VMEM((B, Sq, D), jnp.bfloat16),
                pltpu.SemaphoreType.DMA((4,)),
                pltpu.SemaphoreType.DMA((Hkv,)),
                pltpu.SemaphoreType.DMA((2,)),
                pltpu.SemaphoreType.DMA((2,)),
                pltpu.SemaphoreType.DMA((2,)),
                pltpu.SemaphoreType.DMA((B,)),
            ],
            compiler_params=pltpu.CompilerParams(
                vmem_limit_bytes=100 * 1024 * 1024,
                disable_bounds_checks=NOBC,
                disable_semaphore_checks=NOSC,
            ),
        )(x2, k4, v4, wq, wo)
        return out
    return fn


_impl = build(N=4)


@jax.jit
def pallas_standalone__gqa_block_cached__near_ridge_kernel(
    x: jax.Array,
    k_cache: jax.Array,
    v_cache: jax.Array,
    wq: jax.Array,
    wo: jax.Array,
):
    return _impl(x, k_cache, v_cache, wq, wo)
```

```python
import contextlib
import jax
import jax.numpy as jnp
from jax import lax
import jax.experimental.pallas as pl
import jax.experimental.pallas.tpu as pltpu

_LOG2E = 1.4426950408889634
_NT = (((1,), (1,)), ((), ()))


def build(TK=512, DPOS=1, SH=6, START=1, NOBC=True, NOSC=True, SC=False):
    scope = jax.named_scope if SC else (lambda n: contextlib.nullcontext())

    def fn(x, k_cache, v_cache, wq, wo):
        B, Sq, D = x.shape
        _, Hkv, Sk, Dh = k_cache.shape
        Hq = wq.shape[1] // Dh
        rep = Hq // Hkv
        G = rep * Dh
        M = rep * Sq
        U = B * Hkv
        N = Hkv // 2
        NB = U // N
        NP = (NB - 2) // 2
        NC = Sk // TK
        LT = TK // 128
        HB = B // 2
        HW = Hq * Dh // 2
        scale = (Dh ** -0.5) * _LOG2E
        assert Hkv == 8 and rep == 4 and B % 2 == 0 and Sk % TK == 0 and Dh == 128
        x2 = x.reshape(B * Sq, D)
        k4 = k_cache.reshape(NB, N, Sk, Dh)
        v4 = v_cache.reshape(NB, N, Sk, Dh)

        def kernel(x_hbm, k_hbm, v_hbm, wq_hbm, wo_hbm, out_hbm,
                   x_v, wq_v, wo_v, kbs, kb0, kb1, vb0, vb1, q_scr, s0, s1, m0, m1,
                   oa0, oa1, la0, la1, acc_scr, out_v,
                   sem_x, sem_w0, sem_wq, sem_wo, sem_k, sem_v, sem_o):
            k_bufs = (kb0, kb1, kbs)
            v_bufs = (vb0, vb1)
            s_bufs = (s0, s1)
            m_bufs = (m0, m1)
            o_bufs = (oa0, oa1)
            l_bufs = (la0, la1)

            def x_copy(a):
                rows = pl.ds(a * HB * Sq, HB * Sq)
                return pltpu.make_async_copy(x_hbm.at[rows], x_v.at[rows], sem_x.at[a])

            def wq0_copy(r0, r1):
                cols = pl.ds(r0 * Dh, (r1 - r0) * Dh)
                return pltpu.make_async_copy(wq_hbm.at[:, cols], wq_v.at[0, :, cols], sem_w0.at[r0])

            def wq_copy(h):
                return pltpu.make_async_copy(wq_hbm.at[:, pl.ds(h * G, G)], wq_v.at[h], sem_wq.at[h])

            def wo_copy(a):
                rows = pl.ds(a * HW, HW)
                return pltpu.make_async_copy(wo_hbm.at[rows], wo_v.at[rows], sem_wo.at[a])

            def k_copy(j, slot):
                return pltpu.make_async_copy(k_hbm.at[j], k_bufs[slot], sem_k.at[slot])

            def v_copy(j, slot):
                return pltpu.make_async_copy(v_hbm.at[j], v_bufs[slot], sem_v.at[slot])

            def out_copy(b):
                return pltpu.make_async_copy(out_v.at[b], out_hbm.at[b], sem_o.at[b])

            def qproj(h, b0=0, b1=B, r0=0, r1=rep):
                q = jnp.dot(x_v[b0 * Sq:b1 * Sq, :], wq_v[h, :, r0 * Dh:r1 * Dh],
                            preferred_element_type=jnp.float32)
                q = (q * scale).astype(jnp.bfloat16)
                for bb in range(b0, b1):
                    for r in range(r0, r1):
                        q_scr[bb * Hkv + h, r * Sq:(r + 1) * Sq, :] = (
                            q[(bb - b0) * Sq:(bb - b0 + 1) * Sq, (r - r0) * Dh:(r - r0 + 1) * Dh])

            def b_chunk(j, i, par, kslot, c, mrun):
                cols = slice(c * TK, (c + 1) * TK)
                s = lax.dot_general(q_scr[j * N + i], k_bufs[kslot][i, cols, :], _NT,
                                    preferred_element_type=jnp.float32)
                s_bufs[par][i, :, cols] = s
                t = s[:, 0:128]
                for ii in range(1, LT):
                    t = jnp.maximum(t, s[:, ii * 128:(ii + 1) * 128])
                mrun = t if mrun is None else jnp.maximum(mrun, t)
                if c == NC - 1:
                    m = jnp.max(mrun, axis=1, keepdims=True)
                    m_bufs[par][i] = jnp.broadcast_to(m, (M, 128))
                return mrun, t

            def c_chunk(i, par, c, carry, tok=None):
                lrun, acc = carry
                cols = slice(c * TK, (c + 1) * TK)
                m = m_bufs[par][i]
                if tok is not None:
                    tok = jnp.concatenate([tok[SH * 16:, :]] + [tok[M - 16:, :]] * SH, axis=0)
                    mi = pltpu.bitcast(m, jnp.int32)
                    ti = pltpu.bitcast(tok, jnp.int32)
                    m = pltpu.bitcast(jnp.maximum(mi, jnp.minimum(mi, ti)), jnp.float32)
                p = jnp.exp2(s_bufs[par][i, :, cols] - jnp.concatenate([m] * LT, axis=1))
                t = p[:, 0:128]
                for ii in range(1, LT):
                    t = t + p[:, ii * 128:(ii + 1) * 128]
                lrun = t if lrun is None else lrun + t
                pv = jnp.dot(p.astype(jnp.bfloat16), v_bufs[par][i, cols, :],
                             preferred_element_type=jnp.float32)
                acc = pv if acc is None else pv + acc
                if c == NC - 1:
                    o_bufs[par][i] = acc
                    l_bufs[par][i] = lrun
                return lrun, acc

            def d_unit(par, i, y):
                h = par * N + i
                l = jnp.sum(l_bufs[par][i], axis=1, keepdims=True)
                r0 = pl.reciprocal(l, approx=True)
                r = r0 * (2.0 - l * r0)
                o = (o_bufs[par][i] * r).astype(jnp.bfloat16)
                o = jnp.concatenate([o[rr * Sq:(rr + 1) * Sq, :] for rr in range(rep)], axis=1)
                yi = jnp.dot(o, wo_v[h * G:(h + 1) * G, :], preferred_element_type=jnp.float32)
                return yi if y is None else yi + y

            def d_init(par):
                return acc_scr[...] if par == 1 else None

            def d_finish(j, par, y):
                if par == 0:
                    acc_scr[...] = y
                else:
                    out_v[j // 2] = y.astype(out_v.dtype)
                    out_copy(j // 2).start()

            def body(j, par, first=False, last=False):
                with scope("bwait"):
                    if first:
                        k_copy(0, 2).wait()
                    v_copy(j, par).wait()
                    if not last:
                        k_copy(j + 1, 1 - par).wait()
                if first:
                    for i in range(N):
                        mrun = None
                        for c in range(NC):
                            mrun, _ = b_chunk(0, i, 0, 2, c, mrun)
                y = None if first else d_init(1 - par)
                for i in range(N):
                    mrun = None
                    tok = None
                    carry = (None, None)
                    c_first = i == 0 and not first
                    for c in range(NC):
                        if c_first:
                            carry = c_chunk(i, par, c, carry)
                        if not last:
                            mrun, tok = b_chunk(j + 1, i, 1 - par, 1 - par, c, mrun)
                        if not first and c == DPOS:
                            y = d_unit(1 - par, i, y)
                        if not c_first:
                            carry = c_chunk(i, par, c, carry, tok if first else None)
                if not first:
                    d_finish(j - 1, 1 - par, y)
                if not last:
                    @pl.when(j + 2 < NB)
                    def _():
                        v_copy(j + 2, par).start()

                    @pl.when(j + 3 < NB)
                    def _():
                        k_copy(j + 3, 1 - par).start()

            def pre():
                if START == 0:
                    with scope("p0"):
                        wq0_copy(0, 2).start()
                        x_copy(0).start()
                        x_copy(1).start()
                        wq0_copy(2, 4).start()
                        wq0_copy(0, 2).wait()
                        x_copy(0).wait()
                    for h in range(1, 3):
                        wq_copy(h).start()
                    qproj(0, 0, HB, 0, 2)
                    with scope("qwait"):
                        x_copy(1).wait()
                    for h in range(3, 5):
                        wq_copy(h).start()
                    qproj(0, HB, B, 0, 2)
                    with scope("qwait"):
                        wq0_copy(2, 4).wait()
                    for h in range(5, Hkv):
                        wq_copy(h).start()
                    qproj(0, 0, B, 2, 4)
                elif START == 1:
                    with scope("p0"):
                        wq0_copy(0, 1).start()
                        x_copy(0).start()
                        wq0_copy(1, 3).start()
                        x_copy(1).start()
                        wq0_copy(3, 4).start()
                        wq0_copy(0, 1).wait()
                        x_copy(0).wait()
                    qproj(0, 0, HB, 0, 1)
                    with scope("qwait"):
                        wq0_copy(1, 3).wait()
                    for h in range(1, 3):
                        wq_copy(h).start()
                    qproj(0, 0, HB, 1, 3)
                    with scope("qwait"):
                        x_copy(1).wait()
                        wq0_copy(3, 4).wait()
                    for h in range(3, Hkv):
                        wq_copy(h).start()
                    qproj(0, HB, B, 0, 4)
                    qproj(0, 0, HB, 3, 4)
                else:
                    with scope("p0"):
                        wq0_copy(0, 3).start()
                        x_copy(0).start()
                        x_copy(1).start()
                        wq0_copy(3, 4).start()
                        wq0_copy(0, 3).wait()
                        x_copy(0).wait()
                    for h in range(1, 3):
                        wq_copy(h).start()
                    qproj(0, 0, HB, 0, 3)
                    with scope("qwait"):
                        x_copy(1).wait()
                        wq0_copy(3, 4).wait()
                    for h in range(3, Hkv):
                        wq_copy(h).start()
                    qproj(0, HB, B, 0, 4)
                    qproj(0, 0, HB, 3, 4)
                with scope("qwait"):
                    wq_copy(1).wait()
                qproj(1)

                def qloop(t, c):
                    with scope("qwait"):
                        for hh in range(3):
                            wq_copy(2 + 3 * t + hh).wait()

                    @pl.when(t == 0)
                    def _():
                        k_copy(0, 2).start()
                        k_copy(1, 1).start()
                        v_copy(0, 0).start()

                    @pl.when(t == 1)
                    def _():
                        wo_copy(0).start()
                        v_copy(1, 1).start()
                        k_copy(2, 0).start()
                        wo_copy(1).start()

                    for hh in range(3):
                        qproj(2 + 3 * t + hh)
                    return c

                lax.fori_loop(0, 2, qloop, 0)
                body(0, 0, first=True)
                wo_copy(0).wait()

            def pair(jj):
                body(2 * jj + 1, 1)

                @pl.when(jj == 0)
                def _():
                    wo_copy(1).wait()

                body(2 * jj + 2, 0)

            def post():
                body(NB - 1, 1, last=True)
                y = d_init(1)
                for i in range(N):
                    y = d_unit(1, i, y)
                d_finish(NB - 1, 1, y)
                with scope("final"):
                    for b in range(B):
                        out_copy(b).wait()

            def phase(t, c):
                pl.when(t == 0)(pre)

                @pl.when(jnp.logical_and(t >= 1, t <= NP))
                def _():
                    pair(t - 1)

                pl.when(t == NP + 1)(post)
                return c

            lax.fori_loop(0, NP + 2, phase, 0)

        bf16, f32 = jnp.bfloat16, jnp.float32
        return pl.pallas_call(
            kernel,
            in_specs=[pl.BlockSpec(memory_space=pl.ANY)] * 5,
            out_specs=pl.BlockSpec(memory_space=pl.ANY),
            out_shape=jax.ShapeDtypeStruct((B, Sq, D), x.dtype),
            scratch_shapes=[
                pltpu.VMEM((B * Sq, D), bf16),
                pltpu.VMEM((Hkv, D, G), bf16),
                pltpu.VMEM((Hq * Dh, D), bf16),
                pltpu.VMEM((N, Sk, Dh), bf16),
                pltpu.VMEM((N, Sk, Dh), bf16),
                pltpu.VMEM((N, Sk, Dh), bf16),
                pltpu.VMEM((N, Sk, Dh), bf16),
                pltpu.VMEM((N, Sk, Dh), bf16),
                pltpu.VMEM((U, M, Dh), bf16),
                pltpu.VMEM((N, M, Sk), f32),
                pltpu.VMEM((N, M, Sk), f32),
                pltpu.VMEM((N, M, 128), f32),
                pltpu.VMEM((N, M, 128), f32),
                pltpu.VMEM((N, M, Dh), f32),
                pltpu.VMEM((N, M, Dh), f32),
                pltpu.VMEM((N, M, 128), f32),
                pltpu.VMEM((N, M, 128), f32),
                pltpu.VMEM((Sq, D), f32),
                pltpu.VMEM((B, Sq, D), x.dtype),
                pltpu.SemaphoreType.DMA((2,)),
                pltpu.SemaphoreType.DMA((rep,)),
                pltpu.SemaphoreType.DMA((Hkv,)),
                pltpu.SemaphoreType.DMA((2,)),
                pltpu.SemaphoreType.DMA((3,)),
                pltpu.SemaphoreType.DMA((2,)),
                pltpu.SemaphoreType.DMA((B,)),
            ],
            compiler_params=pltpu.CompilerParams(
                vmem_limit_bytes=96 * 1024 * 1024,
                disable_bounds_checks=NOBC,
                disable_semaphore_checks=NOSC,
            ),
        )(x2, k4, v4, wq, wo)
    return fn


_impl = build()


@jax.jit
def pallas_standalone__gqa_block_cached__near_ridge_kernel(
    x: jax.Array,
    k_cache: jax.Array,
    v_cache: jax.Array,
    wq: jax.Array,
    wo: jax.Array,
):
    return _impl(x, k_cache, v_cache, wq, wo)
```

```python
import jax
import jax.numpy as jnp
from jax import lax
import jax.experimental.pallas as pl
import jax.experimental.pallas.tpu as pltpu

_LOG2E = 1.4426950408889634
_NT = (((1,), (1,)), ((), ()))
_TK = 512
_DPOS = 1
_SH = 6


@jax.jit
def pallas_standalone__gqa_block_cached__near_ridge_kernel(
    x: jax.Array,
    k_cache: jax.Array,
    v_cache: jax.Array,
    wq: jax.Array,
    wo: jax.Array,
):
    B, Sq, D = x.shape
    _, Hkv, Sk, Dh = k_cache.shape
    Hq = wq.shape[1] // Dh
    rep = Hq // Hkv
    G = rep * Dh
    M = rep * Sq
    U = B * Hkv
    N = Hkv // 2
    NB = U // N
    NP = (NB - 2) // 2
    TK = _TK
    NC = Sk // TK
    LT = TK // 128
    HB = B // 2
    HW = Hq * Dh // 2
    scale = (Dh ** -0.5) * _LOG2E
    assert Hkv == 8 and rep == 4 and B % 2 == 0 and Sk % TK == 0 and Dh == 128 and Sq % 16 == 0

    def kernel(x_hbm, k_hbm, v_hbm, wq_hbm, wo_hbm, out_hbm,
               x_v, wq_v, wo_v, kbs, kb0, kb1, vb0, vb1, q_scr, s0, s1, m0, m1,
               oa0, oa1, la0, la1, acc_scr, out_v,
               sem_x, sem_w0, sem_wq, sem_wo, sem_k, sem_v, sem_o):
        k_bufs = (kb0, kb1, kbs)
        v_bufs = (vb0, vb1)
        s_bufs = (s0, s1)
        m_bufs = (m0, m1)
        o_bufs = (oa0, oa1)
        l_bufs = (la0, la1)

        def x_copy(a):
            rows = pl.ds(a * HB * Sq, HB * Sq)
            return pltpu.make_async_copy(x_hbm.at[rows], x_v.at[rows], sem_x.at[a])

        def wq0_copy(r0, r1):
            cols = pl.ds(r0 * Dh, (r1 - r0) * Dh)
            return pltpu.make_async_copy(wq_hbm.at[:, cols], wq_v.at[0, :, cols], sem_w0.at[r0])

        def wq_copy(h):
            return pltpu.make_async_copy(wq_hbm.at[:, pl.ds(h * G, G)], wq_v.at[h], sem_wq.at[h])

        def wo_copy(a):
            rows = pl.ds(a * HW, HW)
            return pltpu.make_async_copy(wo_hbm.at[rows], wo_v.at[rows], sem_wo.at[a])

        def k_copy(j, slot):
            return pltpu.make_async_copy(k_hbm.at[j], k_bufs[slot], sem_k.at[slot])

        def v_copy(j, slot):
            return pltpu.make_async_copy(v_hbm.at[j], v_bufs[slot], sem_v.at[slot])

        def out_copy(b):
            return pltpu.make_async_copy(out_v.at[b], out_hbm.at[b], sem_o.at[b])

        def qproj(h, b0=0, b1=B, r0=0, r1=rep):
            q = jnp.dot(x_v[b0 * Sq:b1 * Sq, :], wq_v[h, :, r0 * Dh:r1 * Dh],
                        preferred_element_type=jnp.float32).astype(jnp.bfloat16)
            for bb in range(b0, b1):
                for r in range(r0, r1):
                    q_scr[bb * Hkv + h, r * Sq:(r + 1) * Sq, :] = (
                        q[(bb - b0) * Sq:(bb - b0 + 1) * Sq, (r - r0) * Dh:(r - r0 + 1) * Dh])

        def b_chunk(j, i, par, kslot, c, mrun):
            cols = slice(c * TK, (c + 1) * TK)
            s = lax.dot_general(q_scr[j * N + i], k_bufs[kslot][i, cols, :], _NT,
                                preferred_element_type=jnp.float32)
            s_bufs[par][i, :, cols] = s
            t = s[:, 0:128]
            for ii in range(1, LT):
                t = jnp.maximum(t, s[:, ii * 128:(ii + 1) * 128])
            mrun = t if mrun is None else jnp.maximum(mrun, t)
            if c == NC - 1:
                m = jnp.max(mrun, axis=1, keepdims=True)
                m_bufs[par][i] = jnp.broadcast_to(m, (M, 128))
            return mrun, t

        def c_chunk(i, par, c, carry, tok=None):
            lrun, acc = carry
            cols = slice(c * TK, (c + 1) * TK)
            m = m_bufs[par][i]
            if tok is not None:
                tok = jnp.concatenate([tok[_SH * 16:, :]] + [tok[M - 16:, :]] * _SH, axis=0)
                mi = pltpu.bitcast(m, jnp.int32)
                ti = pltpu.bitcast(tok, jnp.int32)
                m = pltpu.bitcast(jnp.maximum(mi, jnp.minimum(mi, ti)), jnp.float32)
            z = s_bufs[par][i, :, cols] - jnp.concatenate([m] * LT, axis=1)
            p = jnp.exp2(z * scale)
            t = p[:, 0:128]
            for ii in range(1, LT):
                t = t + p[:, ii * 128:(ii + 1) * 128]
            lrun = t if lrun is None else lrun + t
            pv = jnp.dot(p.astype(jnp.bfloat16), v_bufs[par][i, cols, :],
                         preferred_element_type=jnp.float32)
            acc = pv if acc is None else pv + acc
            if c == NC - 1:
                o_bufs[par][i] = acc
                l_bufs[par][i] = lrun
            return lrun, acc

        def d_unit(par, i, y):
            h = par * N + i
            l = jnp.sum(l_bufs[par][i], axis=1, keepdims=True)
            r0 = pl.reciprocal(l, approx=True)
            r = r0 * (2.0 - l * r0)
            o = (o_bufs[par][i] * r).astype(jnp.bfloat16)
            o = jnp.concatenate([o[rr * Sq:(rr + 1) * Sq, :] for rr in range(rep)], axis=1)
            yi = jnp.dot(o, wo_v[h * G:(h + 1) * G, :], preferred_element_type=jnp.float32)
            return yi if y is None else yi + y

        def d_finish(j, par, y):
            if par == 0:
                acc_scr[...] = y
            else:
                out_v[j // 2] = y.astype(out_v.dtype)
                out_copy(j // 2).start()

        def body(j, par, first=False):
            if first:
                k_copy(0, 2).wait()
            v_copy(j, par).wait()
            k_copy(j + 1, 1 - par).wait()
            if first:
                for i in range(N):
                    mrun = None
                    for c in range(NC):
                        mrun, _ = b_chunk(0, i, 0, 2, c, mrun)
            y = acc_scr[...] if par == 0 and not first else None
            for i in range(N):
                mrun = None
                carry = (None, None)
                c_first = i == 0 and not first
                for c in range(NC):
                    if c_first:
                        carry = c_chunk(i, par, c, carry)
                    mrun, tok = b_chunk(j + 1, i, 1 - par, 1 - par, c, mrun)
                    if not first and c == _DPOS:
                        y = d_unit(1 - par, i, y)
                    if not c_first:
                        carry = c_chunk(i, par, c, carry, tok if first else None)
            if not first:
                d_finish(j - 1, 1 - par, y)

            @pl.when(j + 2 < NB)
            def _():
                v_copy(j + 2, par).start()

            @pl.when(j + 3 < NB)
            def _():
                k_copy(j + 3, 1 - par).start()

        def pre():
            wq0_copy(0, 1).start()
            x_copy(0).start()
            wq0_copy(1, 3).start()
            x_copy(1).start()
            wq0_copy(3, 4).start()
            wq0_copy(0, 1).wait()
            x_copy(0).wait()
            qproj(0, 0, HB, 0, 1)
            wq0_copy(1, 3).wait()
            for h in range(1, 3):
                wq_copy(h).start()
            qproj(0, 0, HB, 1, 3)
            x_copy(1).wait()
            wq0_copy(3, 4).wait()
            for h in range(3, Hkv):
                wq_copy(h).start()
            qproj(0, HB, B, 0, 4)
            qproj(0, 0, HB, 3, 4)
            wq_copy(1).wait()
            qproj(1)

            def qloop(t, c):
                for hh in range(3):
                    wq_copy(2 + 3 * t + hh).wait()

                @pl.when(t == 0)
                def _():
                    k_copy(0, 2).start()
                    k_copy(1, 1).start()
                    v_copy(0, 0).start()

                @pl.when(t == 1)
                def _():
                    wo_copy(0).start()
                    v_copy(1, 1).start()
                    k_copy(2, 0).start()
                    wo_copy(1).start()

                for hh in range(3):
                    qproj(2 + 3 * t + hh)
                return c

            lax.fori_loop(0, 2, qloop, 0)
            body(0, 0, first=True)
            wo_copy(0).wait()

        def pair(jj):
            body(2 * jj + 1, 1)

            @pl.when(jj == 0)
            def _():
                wo_copy(1).wait()

            body(2 * jj + 2, 0)

        def post():
            v_copy(NB - 1, 1).wait()
            y = None
            for i in range(N):
                carry = (None, None)
                for c in range(NC):
                    if c == 1:
                        y = d_unit(0, i, y)
                    if c == NC - 1 and 1 <= i < N - 1:
                        y = d_unit(1, i - 1, y)
                    carry = c_chunk(i, 1, c, carry)
            y = d_unit(1, N - 2, y)
            y = d_unit(1, N - 1, y)
            d_finish(NB - 1, 1, y)
            for b in range(B):
                out_copy(b).wait()

        def phase(t, c):
            pl.when(t == 0)(pre)

            @pl.when(jnp.logical_and(t >= 1, t <= NP))
            def _():
                pair(t - 1)

            pl.when(t == NP + 1)(post)
            return c

        lax.fori_loop(0, NP + 2, phase, 0)

    bf16, f32 = jnp.bfloat16, jnp.float32
    return pl.pallas_call(
        kernel,
        in_specs=[pl.BlockSpec(memory_space=pl.ANY)] * 5,
        out_specs=pl.BlockSpec(memory_space=pl.ANY),
        out_shape=jax.ShapeDtypeStruct((B, Sq, D), x.dtype),
        scratch_shapes=[
            pltpu.VMEM((B * Sq, D), bf16),
            pltpu.VMEM((Hkv, D, G), bf16),
            pltpu.VMEM((Hq * Dh, D), bf16),
            pltpu.VMEM((N, Sk, Dh), bf16),
            pltpu.VMEM((N, Sk, Dh), bf16),
            pltpu.VMEM((N, Sk, Dh), bf16),
            pltpu.VMEM((N, Sk, Dh), bf16),
            pltpu.VMEM((N, Sk, Dh), bf16),
            pltpu.VMEM((U, M, Dh), bf16),
            pltpu.VMEM((N, M, Sk), f32),
            pltpu.VMEM((N, M, Sk), f32),
            pltpu.VMEM((N, M, 128), f32),
            pltpu.VMEM((N, M, 128), f32),
            pltpu.VMEM((N, M, Dh), f32),
            pltpu.VMEM((N, M, Dh), f32),
            pltpu.VMEM((N, M, 128), f32),
            pltpu.VMEM((N, M, 128), f32),
            pltpu.VMEM((Sq, D), f32),
            pltpu.VMEM((B, Sq, D), x.dtype),
            pltpu.SemaphoreType.DMA((2,)),
            pltpu.SemaphoreType.DMA((rep,)),
            pltpu.SemaphoreType.DMA((Hkv,)),
            pltpu.SemaphoreType.DMA((2,)),
            pltpu.SemaphoreType.DMA((3,)),
            pltpu.SemaphoreType.DMA((2,)),
            pltpu.SemaphoreType.DMA((B,)),
        ],
        compiler_params=pltpu.CompilerParams(
            vmem_limit_bytes=96 * 1024 * 1024,
            disable_bounds_checks=True,
            disable_semaphore_checks=True,
        ),
    )(
        x.reshape(B * Sq, D),
        k_cache.reshape(NB, N, Sk, Dh),
        v_cache.reshape(NB, N, Sk, Dh),
        wq,
        wo,
    )
```

```python
import jax
import jax.numpy as jnp
from jax import lax
import jax.experimental.pallas as pl
import jax.experimental.pallas.tpu as pltpu

_LOG2E = 1.4426950408889634
_NT = (((1,), (1,)), ((), ()))
_TK = 512
_DPOS = 1
_SH = 6


@jax.jit
def pallas_standalone__gqa_block_cached__near_ridge_kernel(
    x: jax.Array,
    k_cache: jax.Array,
    v_cache: jax.Array,
    wq: jax.Array,
    wo: jax.Array,
):
    B, Sq, D = x.shape
    _, Hkv, Sk, Dh = k_cache.shape
    Hq = wq.shape[1] // Dh
    rep = Hq // Hkv
    G = rep * Dh
    M = rep * Sq
    U = B * Hkv
    N = Hkv // 2
    NB = U // N
    NP = (NB - 2) // 2
    TK = _TK
    NC = Sk // TK
    LT = TK // 128
    HB = B // 2
    HW = Hq * Dh // 2
    scale = (Dh ** -0.5) * _LOG2E
    assert Hkv == 8 and rep == 4 and B % 2 == 0 and Sk % TK == 0 and Dh == 128 and Sq % 16 == 0

    def kernel(x_hbm, k_hbm, v_hbm, wq_hbm, wo_hbm, out_hbm,
               x_v, wq_v, wo_v, kbs, kb0, kb1, vb0, vb1, q_scr, s0, s1, m0, m1,
               oa0, oa1, la0, la1, acc_scr, out_v,
               sem_x, sem_w0, sem_wq, sem_wo, sem_k, sem_v, sem_o):
        k_bufs = (kb0, kb1, kbs)
        v_bufs = (vb0, vb1)
        s_bufs = (s0, s1)
        m_bufs = (m0, m1)
        o_bufs = (oa0, oa1)
        l_bufs = (la0, la1)

        def x_copy(a):
            rows = pl.ds(a * HB * Sq, HB * Sq)
            return pltpu.make_async_copy(x_hbm.at[rows], x_v.at[rows], sem_x.at[a])

        def wq0_copy(r0, r1):
            cols = pl.ds(r0 * Dh, (r1 - r0) * Dh)
            return pltpu.make_async_copy(wq_hbm.at[:, cols], wq_v.at[0, :, cols], sem_w0.at[r0])

        def wq_copy(h):
            return pltpu.make_async_copy(wq_hbm.at[:, pl.ds(h * G, G)], wq_v.at[h], sem_wq.at[h])

        def wo_copy(a):
            rows = pl.ds(a * HW, HW)
            return pltpu.make_async_copy(wo_hbm.at[rows], wo_v.at[rows], sem_wo.at[a])

        def k_copy(j, slot):
            return pltpu.make_async_copy(k_hbm.at[j], k_bufs[slot], sem_k.at[slot])

        def v_copy(j, slot):
            return pltpu.make_async_copy(v_hbm.at[j], v_bufs[slot], sem_v.at[slot])

        def out_copy(b):
            return pltpu.make_async_copy(out_v.at[b], out_hbm.at[b], sem_o.at[b])

        def qproj(h, b0=0, b1=B, r0=0, r1=rep):
            q = jnp.dot(x_v[b0 * Sq:b1 * Sq, :], wq_v[h, :, r0 * Dh:r1 * Dh],
                        preferred_element_type=jnp.float32).astype(jnp.bfloat16)
            for bb in range(b0, b1):
                for r in range(r0, r1):
                    q_scr[bb * Hkv + h, r * Sq:(r + 1) * Sq, :] = (
                        q[(bb - b0) * Sq:(bb - b0 + 1) * Sq, (r - r0) * Dh:(r - r0 + 1) * Dh])

        def b_chunk(j, i, par, kslot, c, mrun):
            cols = slice(c * TK, (c + 1) * TK)
            s = lax.dot_general(q_scr[j * N + i], k_bufs[kslot][i, cols, :], _NT,
                                preferred_element_type=jnp.float32)
            s_bufs[par][i, :, cols] = s
            t = s[:, 0:128]
            for ii in range(1, LT):
                t = jnp.maximum(t, s[:, ii * 128:(ii + 1) * 128])
            mrun = t if mrun is None else jnp.maximum(mrun, t)
            if c == NC - 1:
                m = jnp.max(mrun, axis=1, keepdims=True)
                m_bufs[par][i] = jnp.broadcast_to(m, (M, 128))
            return mrun, t

        def c_chunk(i, par, c, carry, tok=None):
            lrun, acc = carry
            cols = slice(c * TK, (c + 1) * TK)
            m = m_bufs[par][i]
            if tok is not None:
                tok = jnp.concatenate([tok[_SH * 16:, :]] + [tok[M - 16:, :]] * _SH, axis=0)
                mi = pltpu.bitcast(m, jnp.int32)
                ti = pltpu.bitcast(tok, jnp.int32)
                m = pltpu.bitcast(jnp.maximum(mi, jnp.minimum(mi, ti)), jnp.float32)
            z = s_bufs[par][i, :, cols] - jnp.concatenate([m] * LT, axis=1)
            p = jnp.exp2(z * scale)
            t = p[:, 0:128]
            for ii in range(1, LT):
                t = t + p[:, ii * 128:(ii + 1) * 128]
            lrun = t if lrun is None else lrun + t
            pv = jnp.dot(p.astype(jnp.bfloat16), v_bufs[par][i, cols, :],
                         preferred_element_type=jnp.float32)
            acc = pv if acc is None else pv + acc
            if c == NC - 1:
                o_bufs[par][i] = acc
                l_bufs[par][i] = lrun
            return lrun, acc

        def d_unit(par, i, y):
            h = par * N + i
            l = jnp.sum(l_bufs[par][i], axis=1, keepdims=True)
            r0 = pl.reciprocal(l, approx=True)
            r = r0 * (2.0 - l * r0)
            o = (o_bufs[par][i] * r).astype(jnp.bfloat16)
            o = jnp.concatenate([o[rr * Sq:(rr + 1) * Sq, :] for rr in range(rep)], axis=1)
            yi = jnp.dot(o, wo_v[h * G:(h + 1) * G, :], preferred_element_type=jnp.float32)
            return yi if y is None else yi + y

        def d_finish(j, par, y):
            if par == 0:
                acc_scr[...] = y
            else:
                out_v[j // 2] = y.astype(out_v.dtype)
                out_copy(j // 2).start()

        def body(j, par, first=False):
            if first:
                k_copy(0, 2).wait()
            v_copy(j, par).wait()
            k_copy(j + 1, 1 - par).wait()
            if first:
                for i in range(N):
                    mrun = None
                    for c in range(NC):
                        mrun, _ = b_chunk(0, i, 0, 2, c, mrun)
            y = acc_scr[...] if par == 0 and not first else None
            for i in range(N):
                mrun = None
                carry = (None, None)
                c_first = i == 0 and not first
                for c in range(NC):
                    if c_first:
                        carry = c_chunk(i, par, c, carry)
                    mrun, tok = b_chunk(j + 1, i, 1 - par, 1 - par, c, mrun)
                    if not first and c == _DPOS:
                        y = d_unit(1 - par, i, y)
                    if not c_first:
                        carry = c_chunk(i, par, c, carry, tok if first else None)
            if not first:
                d_finish(j - 1, 1 - par, y)

            @pl.when(j + 2 < NB)
            def _():
                v_copy(j + 2, par).start()

            @pl.when(j + 3 < NB)
            def _():
                k_copy(j + 3, 1 - par).start()

        def pre():
            wq0_copy(0, 1).start()
            x_copy(0).start()
            wq0_copy(1, 3).start()
            x_copy(1).start()
            wq0_copy(3, 4).start()
            wq0_copy(0, 1).wait()
            x_copy(0).wait()
            qproj(0, 0, HB, 0, 1)
            wq0_copy(1, 3).wait()
            for h in range(1, 3):
                wq_copy(h).start()
            qproj(0, 0, HB, 1, 3)
            x_copy(1).wait()
            wq0_copy(3, 4).wait()
            for h in range(3, Hkv):
                wq_copy(h).start()
            qproj(0, HB, B, 0, 4)
            qproj(0, 0, HB, 3, 4)
            wq_copy(1).wait()
            qproj(1)

            def qloop(t, c):
                for hh in range(3):
                    wq_copy(2 + 3 * t + hh).wait()

                @pl.when(t == 0)
                def _():
                    k_copy(0, 2).start()
                    k_copy(1, 1).start()
                    v_copy(0, 0).start()

                @pl.when(t == 1)
                def _():
                    wo_copy(0).start()
                    v_copy(1, 1).start()
                    k_copy(2, 0).start()
                    wo_copy(1).start()

                for hh in range(3):
                    qproj(2 + 3 * t + hh)
                return c

            lax.fori_loop(0, 2, qloop, 0)
            body(0, 0, first=True)
            wo_copy(0).wait()

        def pair(jj):
            body(2 * jj + 1, 1)

            @pl.when(jj == 0)
            def _():
                wo_copy(1).wait()

            body(2 * jj + 2, 0)

        def post():
            v_copy(NB - 1, 1).wait()
            y = None
            for i in range(N):
                carry = (None, None)
                for c in range(NC):
                    if c == 1:
                        y = d_unit(0, i, y)
                    if c == NC - 1 and 1 <= i < N - 1:
                        y = d_unit(1, i - 1, y)
                    carry = c_chunk(i, 1, c, carry)
            y = d_unit(1, N - 2, y)
            y = d_unit(1, N - 1, y)
            d_finish(NB - 1, 1, y)
            for b in range(B):
                out_copy(b).wait()

        def steady():
            def pair_step(jj, c):
                pair(jj)
                return c

            lax.fori_loop(0, NP, pair_step, 0)

        def phase(t, c):
            pl.when(t == 0)(pre)
            pl.when(t == 1)(steady)
            pl.when(t == 2)(post)
            return c

        lax.fori_loop(0, 3, phase, 0)

    bf16, f32 = jnp.bfloat16, jnp.float32
    return pl.pallas_call(
        kernel,
        in_specs=[pl.BlockSpec(memory_space=pl.ANY)] * 5,
        out_specs=pl.BlockSpec(memory_space=pl.ANY),
        out_shape=jax.ShapeDtypeStruct((B, Sq, D), x.dtype),
        scratch_shapes=[
            pltpu.VMEM((B * Sq, D), bf16),
            pltpu.VMEM((Hkv, D, G), bf16),
            pltpu.VMEM((Hq * Dh, D), bf16),
            pltpu.VMEM((N, Sk, Dh), bf16),
            pltpu.VMEM((N, Sk, Dh), bf16),
            pltpu.VMEM((N, Sk, Dh), bf16),
            pltpu.VMEM((N, Sk, Dh), bf16),
            pltpu.VMEM((N, Sk, Dh), bf16),
            pltpu.VMEM((U, M, Dh), bf16),
            pltpu.VMEM((N, M, Sk), f32),
            pltpu.VMEM((N, M, Sk), f32),
            pltpu.VMEM((N, M, 128), f32),
            pltpu.VMEM((N, M, 128), f32),
            pltpu.VMEM((N, M, Dh), f32),
            pltpu.VMEM((N, M, Dh), f32),
            pltpu.VMEM((N, M, 128), f32),
            pltpu.VMEM((N, M, 128), f32),
            pltpu.VMEM((Sq, D), f32),
            pltpu.VMEM((B, Sq, D), x.dtype),
            pltpu.SemaphoreType.DMA((2,)),
            pltpu.SemaphoreType.DMA((rep,)),
            pltpu.SemaphoreType.DMA((Hkv,)),
            pltpu.SemaphoreType.DMA((2,)),
            pltpu.SemaphoreType.DMA((3,)),
            pltpu.SemaphoreType.DMA((2,)),
            pltpu.SemaphoreType.DMA((B,)),
        ],
        compiler_params=pltpu.CompilerParams(
            vmem_limit_bytes=96 * 1024 * 1024,
            disable_bounds_checks=True,
            disable_semaphore_checks=True,
        ),
    )(
        x.reshape(B * Sq, D),
        k_cache.reshape(NB, N, Sk, Dh),
        v_cache.reshape(NB, N, Sk, Dh),
        wq,
        wo,
    )
```
